```python
import os as _os
_os.environ.setdefault("JAX_PLATFORMS", "cpu")
import jax
import jax.numpy as jnp

def _softmax(x, axis=-1):
    return jax.nn.softmax(x, axis=axis)
def _gelu(x):
    return jax.nn.gelu(x, approximate=True)
def _silu(x):
    return jax.nn.silu(x)
def _sigmoid(x):
    return jax.nn.sigmoid(x)
def _layernorm(x, axis=-1, eps=1e-5):
    m = jnp.mean(x, axis=axis, keepdims=True)
    v = jnp.var(x, axis=axis, keepdims=True)
    return (x - m) / jnp.sqrt(v + eps)
def _scatter_add(tgt, idx, src, axis=0):
    return tgt.at[idx].add(src)
def _segment_sum(src, seg, n):
    return jax.ops.segment_sum(src, seg, n)
class _Rng:
    def __init__(self, key):
        self._k = key
    def _next(self):
        self._k, sub = jax.random.split(self._k)
        return sub
    def normal(self, shape):
        return jax.random.normal(self._next(), shape, dtype=jnp.bfloat16)
    def randint(self, lo, hi, shape):
        return jax.random.randint(self._next(), shape, lo, hi, dtype=jnp.int32)
    def uniform(self, shape, lo=0.0, hi=1.0):
        return jax.random.uniform(self._next(), shape, jnp.bfloat16, lo, hi)
    def permutation(self, n):
        return jax.random.permutation(self._next(), n)


kernel_name = 'interleave_layers__mha_block__mixer_s_mlp__prompt'

def setup_inputs():
    _rng = _Rng(jax.random.key(int.from_bytes(__import__("os").urandom(4), "little")))
    _w = (lambda a: (lambda t: t.astype(jnp.bfloat16) if jnp.issubdtype(t.dtype, jnp.floating) else t)(jnp.asarray(a)))
    def _A_setup():
        B, S, D, H = 1, 2048, 448, 16
        return {
            "x": _w((lambda *s: _rng.normal(s) * 0.05)(B, S, D)),
            "wqkv": _w((lambda *s: _rng.normal(s) * 0.05)(D, 3 * D)),
            "wo": _w((lambda *s: _rng.normal(s) * 0.05)(D, D)),
        }
    _A_in = _A_setup()

    def _B_setup():
        B, S, D, F = 1, 2048, 448, 1792
        return {
            "x":  _w((lambda *s: _rng.normal(s) * 0.05)(B, S, D)),
            "w1": _w((lambda *s: _rng.normal(s) * 0.8)(D, D) * (D ** -0.5)),
            "w2": _w((lambda *s: _rng.normal(s) * 0.8)(D, D) * (D ** -0.5)),
            "w3": _w((lambda *s: _rng.normal(s) * 0.8)(D, F) * (D ** -0.5)),
            "w4": _w((lambda *s: _rng.normal(s) * 0.8)(F, D) * (F ** -0.5)),
        }
    _B_in = _B_setup()

    return {
        "A_x": _A_in["x"],
        "A_wqkv": _A_in["wqkv"],
        "A_wo": _A_in["wo"],
        "B_x": _B_in["x"],
        "B_w1": _B_in["w1"],
        "B_w2": _B_in["w2"],
        "B_w3": _B_in["w3"],
        "B_w4": _B_in["w4"],
    }

def reference(A_x, A_wqkv, A_wo, B_x, B_w1, B_w2, B_w3, B_w4):
    def _A_ref(x, wqkv, wo):
        B, S, D = x.shape
        H = 16
        Dh = D // H
        qkv = (lambda x, *d: x.transpose(*d))((x @ wqkv).reshape(B, S, 3, H, Dh), 2, 0, 3, 1, 4)
        q, k, v = qkv[0], qkv[1], qkv[2]
        scores = jnp.einsum("bhqd,bhkd->bhqk", q, k) * (Dh ** -0.5)
        p = _softmax(scores, axis=-1)
        o = jnp.einsum("bhqk,bhkd->bhqd", p, v)
        return (lambda x, *d: x.transpose(*d))(o, 0, 2, 1, 3).reshape(B, S, D) @ wo

    def _B_ref(x, w1, w2, w3, w4):
        B, S, D = x.shape
        h = _gelu(_layernorm(x, axis=-1) @ w1)
        c = D // 4
        g0 = jnp.pad(h[:, :, 0*c:1*c], ((0, 0), (1, 0), (0, 0)))[:, :S, :]
        g1 = jnp.pad(h[:, :, 1*c:2*c], ((0, 0), (0, 1), (0, 0)))[:, 1:, :]
        g2 = jnp.pad(h[:, :, 2*c:3*c], ((0, 0), (2, 0), (0, 0)))[:, :S, :]
        g3 = jnp.pad(h[:, :, 3*c:   ], ((0, 0), (0, 2), (0, 0)))[:, 2:, :]
        hs = jnp.concatenate([g0, g1, g2, g3], axis=-1) @ w2
        x1 = x + hs
        h2 = _gelu(_layernorm(x1, axis=-1) @ w3) @ w4
        return x1 + h2

    x = A_x
    x = x + _A_ref(_layernorm(x, axis=-1), A_wqkv, A_wo)
    x = x + _B_ref(_layernorm(x, axis=-1), B_w1, B_w2, B_w3, B_w4)
    x = x + _A_ref(_layernorm(x, axis=-1), A_wqkv, A_wo)
    x = x + _B_ref(_layernorm(x, axis=-1), B_w1, B_w2, B_w3, B_w4)
    return x
```

```python
import math

import jax
import jax.numpy as jnp
from jax import lax
import jax.experimental.pallas as pl
import jax.experimental.pallas.tpu as pltpu

S = 2048
D = 448
H = 16
DH = D // H
F = 1792
T = 512
NB = S // T
KC = 128
LANE = 128
EPS = 1e-5
QSCALE = (DH ** -0.5) * math.log2(math.e)
GELU_C1 = math.sqrt(2.0 / math.pi)
GELU_C2 = GELU_C1 * 0.044715

f32 = jnp.float32
bf16 = jnp.bfloat16


def _dot(a, b):
    return jnp.dot(a, b, preferred_element_type=f32)


def _layernorm(x):
    m = jnp.sum(x, axis=0, keepdims=True) * (1.0 / D)
    c = x - m
    v = jnp.sum(c * c, axis=0, keepdims=True) * (1.0 / D)
    return c * lax.rsqrt(v + EPS)


def _gelu(x):
    t = jnp.tanh(x * (GELU_C1 + GELU_C2 * (x * x)))
    hx = 0.5 * x
    return hx + hx * t


def _group_start(g):
    return min(4 * DH * g, D - LANE)


def _head_window(h):
    return (DH * h, 0) if h % 2 == 0 else (DH * h - 4, 4)


def _kernel(x_hbm, wqkv_hbm, wo_hbm, w1_hbm, w2_hbm, w3_hbm, w4t_hbm, out_hbm,
            xin, wqkv_s, wo_s, w1_s, w2_s, w3_s, w4t,
            wqkvt, wot, w1t, w2t, w3t,
            xs, ys, hs, qt, kn, vt, ot, sc, mx, obuf, in_sem, out_sem):
    def blk(j):
        return slice(j * T, (j + 1) * T)

    x_copies = [pltpu.make_async_copy(x_hbm.at[:, blk(j)], xin.at[:, blk(j)], in_sem.at[j])
                for j in range(NB)]
    w_copies = [pltpu.make_async_copy(src, dst, in_sem.at[NB + i])
                for i, (src, dst) in enumerate(
                    [(wqkv_hbm, wqkv_s), (wo_hbm, wo_s), (w1_hbm, w1_s), (w2_hbm, w2_s),
                     (w3_hbm, w3_s), (w4t_hbm, w4t)])]
    out_copies = [pltpu.make_async_copy(obuf.at[:, blk(j)], out_hbm.at[:, blk(j)], out_sem.at[j])
                  for j in range(NB)]

    w_copies[0].start()
    for c in x_copies:
        c.start()
    for c in w_copies[1:]:
        c.start()

    hs[:, 0:LANE] = jnp.zeros((D, LANE), bf16)
    hs[:, LANE + S:] = jnp.zeros((D, LANE), bf16)

    def transpose_weight(src, dst, n):
        for c in range(0, n, LANE):
            w = min(LANE, n - c)
            dst[c:c + w, :] = src[:, c:c + w].T

    def transpose_wo():
        row = lax.broadcasted_iota(jnp.int32, (32, D), 0)
        w = wo_s[...].astype(f32)
        parts = []
        for h in range(H):
            start, first = _head_window(h)
            own = (row >= first) & (row < first + DH)
            parts.append(jnp.where(own, w[start:start + 32, :], 0.0))
        wp = jnp.concatenate(parts, axis=0).astype(bf16)
        for c in range(0, D, LANE):
            wd = min(LANE, D - c)
            wot[c:c + wd, :] = wp[:, c:c + wd].T

    def qkv_block(j, x):
        xn = _layernorm(x).astype(bf16)
        q = _dot(wqkvt[0:D, :], xn)
        qt[:, blk(j)] = (q * QSCALE).astype(bf16)
        k = _dot(wqkvt[D:2 * D, :], xn).astype(bf16)
        for g in range(4):
            s0 = _group_start(g)
            kn[g, blk(j), :] = k[s0:s0 + LANE, :].T
        v = _dot(wqkvt[2 * D:3 * D, :], xn)
        row = lax.broadcasted_iota(jnp.int32, (32, T), 0)
        for h in range(H):
            start, first = _head_window(h)
            own = (row >= first) & (row < first + DH)
            vt[h, :, blk(j)] = jnp.where(own, v[start:start + 32, :], 1.0).astype(bf16)

    def attend(h1, h2):
        for j in range(NB):
            if h1 is not None:
                g = h1 // 4
                s0 = jnp.minimum(4 * DH * g, D - LANE)
                q = qt[pl.ds(pl.multiple_of(s0, 16), LANE), blk(j)]
                row = lax.broadcasted_iota(jnp.int32, (LANE, T), 0)
                lo = DH * h1 - s0
                qm = jnp.where((row >= lo) & (row < lo + DH), q.astype(f32), 0.0).astype(bf16)
                m_new = None
            if h2 is not None:
                m = mx[j]
                acc = None
            for c in range(S // KC):
                rows = slice(c * KC, (c + 1) * KC)
                if h2 is not None:
                    d = sc[j, rows, :].reshape(KC // 8, 8, T) - m[None]
                    p = jnp.exp2(d).reshape(KC, T).astype(bf16)
                    o = _dot(vt[h2, :, rows], p)
                    acc = o if acc is None else acc + o
                if h1 is not None:
                    s = _dot(kn[g, rows, :], qm)
                    sc[j, rows, :] = s
                    t = jnp.max(s.reshape(KC // 8, 8, T), axis=0)
                    m_new = t if m_new is None else jnp.maximum(m_new, t)
            if h1 is not None:
                mx[j] = jnp.broadcast_to(jnp.max(m_new, axis=0, keepdims=True), (8, T))
            if h2 is not None:
                l = jnp.where(h2 % 2 == 0, acc[DH:DH + 1, :], acc[0:1, :])
                ot[h2, :, blk(j)] = (acc * (1.0 / l)).astype(bf16)

    def attention():
        attend(0, None)

        def body(i, carry):
            attend(i + 1, i)
            return carry

        lax.fori_loop(0, H - 1, body, 0)
        attend(None, H - 1)

    def mixer_in(j):
        o = ot[:, :, blk(j)].reshape(H * 32, T)
        x = xs[:, blk(j)] + _dot(wot[...], o)
        xs[:, blk(j)] = x
        y = _layernorm(x)
        ys[:, blk(j)] = y
        h = _gelu(_dot(w1t[...], _layernorm(y).astype(bf16)))
        hs[:, LANE + j * T:LANE + (j + 1) * T] = h.astype(bf16)

    def mixer_out(j):
        c = D // 4
        base = LANE + j * T
        g = jnp.concatenate(
            [hs[i * c:(i + 1) * c, base + off:base + off + T]
             for i, off in enumerate((-1, 1, -2, 2))], axis=0)
        x1 = ys[:, blk(j)] + _dot(w2t[...], g)
        z = _layernorm(x1).astype(bf16)
        u = _gelu(_dot(w3t[...], z)).astype(bf16)
        x = xs[:, blk(j)] + (x1 + _dot(w4t[...], u))
        return x

    w_copies[0].wait()
    transpose_weight(wqkv_s, wqkvt, 3 * D)
    for j in range(NB):
        x_copies[j].wait()
        xs[:, blk(j)] = xin[:, blk(j)].astype(f32)

    def layer(l, carry):
        for j in range(NB):
            qkv_block(j, xs[:, blk(j)])
        attention()

        @pl.when(l == 0)
        def _():
            for c in w_copies[1:]:
                c.wait()
            transpose_wo()
            transpose_weight(w1_s, w1t, D)
            transpose_weight(w2_s, w2t, D)
            transpose_weight(w3_s, w3t, F)

        for j in range(NB):
            mixer_in(j)
        for j in range(NB):
            xs[:, blk(j)] = mixer_out(j)
        return carry

    lax.fori_loop(0, 2, layer, 0)

    for j in range(NB):
        obuf[:, blk(j)] = xs[:, blk(j)].astype(bf16)
        out_copies[j].start()
    for c in out_copies:
        c.wait()


@jax.jit
def pallas_interleave_layers__mha_block__mixer_s_mlp__prompt_kernel(
    A_x: jax.Array,
    A_wqkv: jax.Array,
    A_wo: jax.Array,
    B_x: jax.Array,
    B_w1: jax.Array,
    B_w2: jax.Array,
    B_w3: jax.Array,
    B_w4: jax.Array,
):
    del B_x
    vmem = pltpu.VMEM
    out_t = pl.pallas_call(
        _kernel,
        out_shape=jax.ShapeDtypeStruct((D, S), bf16),
        in_specs=[pl.BlockSpec(memory_space=pl.ANY)] * 7,
        out_specs=pl.BlockSpec(memory_space=pl.ANY),
        scratch_shapes=[
            vmem((D, S), bf16),
            vmem((D, 3 * D), bf16),
            vmem((D, D), bf16),
            vmem((D, D), bf16),
            vmem((D, D), bf16),
            vmem((D, F), bf16),
            vmem((D, F), bf16),
            vmem((3 * D, D), bf16),
            vmem((D, H * 32), bf16),
            vmem((D, D), bf16),
            vmem((D, D), bf16),
            vmem((F, D), bf16),
            vmem((D, S), f32),
            vmem((D, S), f32),
            vmem((D, S + 2 * LANE), bf16),
            vmem((D, S), bf16),
            vmem((4, S, LANE), bf16),
            vmem((H, 32, S), bf16),
            vmem((H, 32, S), bf16),
            vmem((NB, S, T), f32),
            vmem((NB, 8, T), f32),
            vmem((D, S), bf16),
            pltpu.SemaphoreType.DMA((NB + 6,)),
            pltpu.SemaphoreType.DMA((NB,)),
        ],
        compiler_params=pltpu.CompilerParams(vmem_limit_bytes=100 * 1024 * 1024),
    )(A_x.reshape(S, D).T, A_wqkv, A_wo, B_w1, B_w2, B_w3, B_w4.T)
    return out_t.T.reshape(1, S, D)
```

```python
import math

import jax
import jax.numpy as jnp
from jax import lax
import jax.experimental.pallas as pl
import jax.experimental.pallas.tpu as pltpu

S = 2048
D = 448
H = 16
DH = D // H
F = 1792
T = 512
NB = S // T
LANE = 128
NT = T // LANE
KC = 128
D2 = D // 2
F2 = F // 2
T2 = T // 2
EPS = 1e-5
QSCALE = (DH ** -0.5) * math.log2(math.e)
GELU_C1 = math.sqrt(2.0 / math.pi)
GELU_K = (GELU_C1 * 0.044715) ** (1.0 / 3.0)
GELU_A = GELU_C1 / GELU_K

GROUP = D // 4
SHIFTS = (1, -1, 2, -2)
UNROLL = 3

RC_Q = (224,)
RC_KV = (112, 112)
RC_AO = (224,)
RC_MI = (224,)
RC_MO = (176, 48)
RC_F = (192,) + (32,) * 22
RC_F_LAST = (128,) + (48,) * 16
RC_F_FIRST = (128,) * 7
RC_DOWN = (64, 64, 48, 48)
RC_DOWN_LAST = (48, 48, 48, 48, 32)

PLAN = ("ao0 ao1 epi0 mi0 mi1 epi1 mo0 up0; epi2 epi3 / dn0; ao2 ao3; mi2 / qk0; mi3 mo1 mo2 "
        "up1 mo3 up2 dn1 up3 dn2 dn3 qk1 qk2 qk3")
PLAN_LAST = ("ao1 ao0 epi1 mi0 mi1 mo0 epi0 up0; epi2 epi3 / dn0; ao2 ao3 mi2; mi3 / mo1; mo2 up1 "
             "up2 mo3 dn1 up3 dn2 dn3")

f32 = jnp.float32
bf16 = jnp.bfloat16

LHS_TERMS = ((1, 0, 3), (1, 2, 3), (0, 0, 0), (0, 3, 3), (1, 0, 1), (-1, 2, 0), (-1, 1, 3))
RHS_TERMS = ((1, 0, 3), (0, 0, 0), (-1, 1, 3), (-1, 2, 0), (0, 3, 3), (1, 0, 1), (1, 2, 3))


def _term(spec, quadrant):
    sign, first, second = spec
    if sign == 0:
        return quadrant(first)
    return quadrant(first) + quadrant(second) if sign > 0 else quadrant(first) - quadrant(second)


def _dot(a, b):
    return jnp.dot(a, b, preferred_element_type=f32)


def _gelu_scaled(y):
    return y + y * jnp.tanh(y * (y * y + GELU_A))


def _reciprocal(x):
    r = pl.reciprocal(x, approx=True)
    return r * (2.0 - x * r)


def _lane_tiles(x):
    return [x[:, c:c + LANE] for c in range(0, x.shape[1], LANE)]


class _Tiles:
    def __init__(self, ref):
        self.ref = ref

    def __getitem__(self, idx):
        return self.ref[idx]

    def __setitem__(self, idx, val):
        self.ref[idx] = val.astype(bf16)

    def wide(self, i, rows=slice(None)):
        return jnp.concatenate([self.ref[i, t, rows, :] for t in range(self.ref.shape[1])], axis=1)


def _strassen(lhs, rhs, chunks, emit):
    r0 = 0
    for n in chunks:
        rows = slice(r0, r0 + n)
        r0 += n

        def prod(i):
            a, b = lhs(i, rows), rhs(i)
            pad = a.shape[1] - b.shape[0]
            if pad:
                b = jnp.concatenate([b, jnp.zeros((pad, b.shape[1]), b.dtype)], axis=0)
            return _dot(a.astype(bf16), b.astype(bf16))

        m3 = prod(2)
        yield
        m5 = prod(4)
        emit(1, rows, m3 + m5)
        yield
        m4 = prod(3)
        c11 = m4 - m5
        yield
        m2 = prod(1)
        emit(2, rows, m2 + m4)
        c22 = m3 - m2
        yield
        m1 = prod(0)
        c11 = c11 + m1
        c22 = c22 + m1
        yield
        emit(0, rows, c11 + prod(6))
        yield
        emit(3, rows, c22 + prod(5))
        yield


def _run(*gens):
    for g in gens:
        for _ in g:
            pass


def _chain(*gens):
    for g in gens:
        yield from g


def _weave(main, n_main, side, n_side):
    done = 0
    for i, _ in enumerate(main):
        while done * n_main < (i + 1) * n_side:
            next(side, None)
            done += 1
    _run(side)


def _group_start(g):
    return (g // 2) * D2 + (g % 2) * (D2 - LANE)


def _head_window(h):
    return (DH * h, 0) if h % 2 == 0 else (DH * h - 4, 4)


def _query_rows(h):
    lo = DH * h - _group_start(h // 4)
    return lo, lo // 16 * 16, -(-(lo + DH) // 16) * 16


def _kernel(x_hbm, wqkv_hbm, wo_hbm, w1_hbm, w2_hbm, w3_hbm, w4t_hbm, out_hbm,
            sc, mx, qt, kn, vt, ot,
            xin, wq_s, wk_s, wv_s, wo_s, w1_s, w2_s, w3_s, w4t_s,
            wqkvc, woc, w1c, w2c, w3c, w4c,
            xs, ys, hs, us, rs, kf, qf, vf, obuf, stats, in_sem, out_sem):
    qt, kn, vt, wqkvc, woc, w1c, w2c, w3c, w4c, hs, us, rs = map(
        _Tiles, (qt, kn, vt, wqkvc, woc, w1c, w2c, w3c, w4c, hs, us, rs))

    def blk(j):
        return slice(j * T, (j + 1) * T)

    def quad(q, rows=slice(0, D2)):
        r0, c0 = (q // 2) * D2, (q % 2) * T2
        return slice(r0 + rows.start, r0 + rows.stop), slice(c0, c0 + T2)

    x_copies = [pltpu.make_async_copy(x_hbm.at[:, blk(j)], xin.at[j], in_sem.at[j])
                for j in range(NB)]
    cuts = (0, 4 * LANE, 2 * D, 3 * D)
    w_copies = [pltpu.make_async_copy(src, dst, in_sem.at[NB + i])
                for i, (src, dst) in enumerate(
                    [(wqkv_hbm.at[:, lo:hi], w)
                     for lo, hi, w in zip(cuts, cuts[1:], (wq_s, wk_s, wv_s))]
                    + [(wo_hbm, wo_s), (w1_hbm, w1_s), (w2_hbm, w2_s), (w3_hbm, w3_s),
                       (w4t_hbm, w4t_s)])]
    out_copies = {}

    def send(j, rows):
        sem = out_sem.at[len(out_copies)]
        out_copies[j, rows.start] = pltpu.make_async_copy(
            obuf.at[j, rows, :], out_hbm.at[rows, blk(j)], sem)
        out_copies[j, rows.start].start()

    class Weight:
        def __init__(self, store, quadrant):
            self.store, self.quadrant = store, quadrant
            self.rows_done, self.quads = {}, {}

        def lhs(self, part=0):
            def get(i, rows):
                item = 7 * part + i
                if rows.stop <= self.rows_done.get(item, 0):
                    return self.store.wide(item, rows)
                self.rows_done[item] = rows.stop

                def quadrant(q):
                    key = (part, q, rows.start)
                    if key not in self.quads:
                        self.quads[key] = self.quadrant(part, q, rows)
                    return self.quads[key]
                term = _term(LHS_TERMS[i], quadrant)
                for c, t in enumerate(_lane_tiles(term)):
                    self.store[item, c, rows, :] = t
                return term
            return get

    def transposing(columns, n2, scales):
        done = {}

        def tile(k, c):
            if (k, c) not in done:
                w = columns(k, c)
                if w.shape[0] % LANE:
                    pad = jnp.zeros((LANE - w.shape[0] % LANE, w.shape[1]), w.dtype)
                    w = jnp.concatenate([w, pad], axis=0)
                done[k, c] = w.T.astype(f32)
            return done[k, c]

        def quadrant(part, q, rows):
            lo = (2 * part + q // 2) * n2 + rows.start
            hi = lo + rows.stop - rows.start
            w = jnp.concatenate(
                [tile(q % 2, c)[max(lo - c * LANE, 0):min(hi - c * LANE, LANE)]
                 for c in range(lo // LANE, (hi - 1) // LANE + 1)], axis=0)
            return w if scales[part] is None else w * scales[part]
        return quadrant

    def columns_of(ref):
        return lambda k, c: ref[k * D2:(k + 1) * D2, c * LANE:min((c + 1) * LANE, ref.shape[1])]

    def wqkv_columns(k, c):
        ref, c0 = (wq_s, 0) if c < 4 else (wk_s, 4) if c < 7 else (wv_s, 7)
        return columns_of(ref)(k, c - c0)

    def wo_columns(k, c):
        w = columns_of(wo_s)(k, c).astype(f32)
        row = lax.broadcasted_iota(jnp.int32, (32, w.shape[1]), 0)
        parts = []
        for h in range(H // 2):
            start, first = _head_window(h)
            parts.append(jnp.where((row >= first) & (row < first + DH), w[start:start + 32], 0.0))
        return jnp.concatenate(parts, axis=0).astype(bf16)

    def w4_quadrant(part, q, rows):
        r0, c0 = (q // 2) * D2, (q % 2) * F2
        return w4t_s[r0 + rows.start:r0 + rows.stop, c0:c0 + F2].astype(f32) * (0.5 / GELU_K)

    wqkv = Weight(wqkvc, transposing(wqkv_columns, D2, (QSCALE, None, None)))
    wo = Weight(woc, transposing(wo_columns, D2, (None,)))
    w1 = Weight(w1c, transposing(columns_of(w1_s), D2, (GELU_K,)))
    w2 = Weight(w2c, transposing(columns_of(w2_s), D2, (0.5 / GELU_K,)))
    w3 = Weight(w3c, transposing(columns_of(w3_s), F2, (GELU_K,)))
    w4 = Weight(w4c, w4_quadrant)

    def clear_q():
        for h in range(H):
            _, r0, r1 = _query_rows(h)
            for a, b in ((0, r0), (r1, LANE)):
                if b > a:
                    row = lax.broadcasted_iota(jnp.int32, (b - a, LANE), 0)
                    for t in range(S // LANE):
                        qt[h, t, a:b, :] = jnp.where(row < 0, 1.0, 0.0)

    class Stats:
        def __init__(self):
            self.part = {}

        def add(self, side, x):
            x = x.reshape(x.shape[0] // 8, 8, x.shape[1])
            new = jnp.sum(x, axis=0), jnp.sum(x * x, axis=0)
            old = self.part.get(side)
            self.part[side] = new if old is None else (old[0] + new[0], old[1] + new[1])

        def save(self, slot, twice=False):
            s1, s2 = [jnp.concatenate([self.part[side][i] for side in sorted(self.part)], axis=1)
                      for i in range(2)]
            m = jnp.sum(s1, axis=0, keepdims=True) * (1.0 / D)
            v = jnp.maximum(jnp.sum(s2, axis=0, keepdims=True) * (1.0 / D) - m * m, 0.0)
            r = lax.rsqrt(v + EPS)
            stats[slot, 0] = jnp.broadcast_to(m, (8, T))
            stats[slot, 1] = jnp.broadcast_to(r, (8, T))
            if twice:
                stats[slot, 2] = jnp.broadcast_to(r * lax.rsqrt(v * r * r + EPS), (8, T))

    def normed(ref, j, slot, scale, r, c):
        x = ref[j, r, c]
        n = x.shape[0]
        x = (x.reshape(n // 8, 8, T2) - stats[slot, 0, :, c][None]) * stats[slot, scale, :, c][None]
        return x.reshape(n, T2)

    def factors(quadrant, keep=None):
        built = {}

        def rhs(i):
            if i in built:
                return rs.wide(7 * keep + i, built[i])
            term = _term(RHS_TERMS[i], quadrant)
            if keep is not None:
                built[i] = slice(0, term.shape[0])
                for a, t in enumerate(_lane_tiles(term)):
                    rs[7 * keep + i, a, built[i], :] = t
            return term
        return rhs

    def qkv(j):
        rhs = factors(lambda q: normed(xs, j, j, 1, *quad(q)), 0)

        def into(ref):
            def emit(q, rows, v):
                ref[quad(q, rows)] = v
            return emit
        yield from _strassen(wqkv.lhs(0), rhs, RC_Q, into(qf))
        for h in range(H):
            lo, r0, r1 = _query_rows(h)
            s0 = _group_start(h // 4)
            row = lax.broadcasted_iota(jnp.int32, (r1 - r0, T), 0) + r0
            q = jnp.where((row >= lo) & (row < lo + DH), qf[s0 + r0:s0 + r1, :], 0.0)
            for a, t in enumerate(_lane_tiles(q)):
                qt[h, j * NT + a, r0:r1, :] = t
        yield from _strassen(wqkv.lhs(1), rhs, RC_KV, into(kf))
        for g in range(4):
            s0 = _group_start(g)
            kn[g, blk(j), :] = kf[s0:s0 + LANE, :].astype(bf16).T
        yield from _strassen(wqkv.lhs(2), rhs, RC_KV, into(vf))
        row = lax.broadcasted_iota(jnp.int32, (32, T), 0)
        for h in range(H):
            start, first = _head_window(h)
            own = (row >= first) & (row < first + DH)
            v = jnp.where(own, vf[start:start + 32, :], 1.0)
            for a, t in enumerate(_lane_tiles(v)):
                vt[h, j * NT + a] = t
    N_QKV = 7 * (len(RC_Q) + 2 * len(RC_KV))

    def attend(h1, j1, h2, j2, slot, odd=False):
        if h1 is not None:
            g = h1 // 4
            qm = jnp.concatenate([qt[h1, j1 * NT + a] for a in range(NT)], axis=1)
            m_new = None
        if h2 is not None:
            m = jnp.broadcast_to(jnp.max(mx[slot], axis=0, keepdims=True), (8, T))
            acc = None
        for c in range(S // KC):
            rows = slice(c * KC, (c + 1) * KC)
            if h2 is not None:
                d = sc[slot, rows, :].reshape(KC // 8, 8, T) - m[None]
                p = jnp.exp2(d).reshape(KC, T).astype(bf16)
            if h1 is not None:
                s = _dot(kn[g, rows, :], qm)
            if h2 is not None:
                o = _dot(vt[h2, c], p)
                acc = o if acc is None else acc + o
            if h1 is not None:
                sc[slot, rows, :] = s
                t = jnp.max(s.reshape(KC // 8, 8, T), axis=0)
                m_new = t if m_new is None else jnp.maximum(m_new, t)
            yield
        if h1 is not None:
            mx[slot] = m_new
        if h2 is not None:
            ot[j2, h2] = acc * _reciprocal(acc[0:1, :] if odd else acc[DH:DH + 1, :])
    N_ATT = S // KC

    def pair(i):
        h, j = (2 * i) % H, (2 * i) // H * 2
        hn, jn = (2 * i + 2) % H, (2 * i + 2) // H * 2
        _run(attend(h + 1, j, h, j, 0), attend(h + 1, j + 1, h, j + 1, 1),
             attend(hn, jn, h + 1, j, 0, odd=True),
             attend(hn, jn + 1, h + 1, j + 1, 1, odd=True))

    def tail(n):
        j = NB - 2 + n % 2
        if n < 2:
            return attend(H - 1, j, H - 2, j, n % 2)
        return attend(None, None, H - 1, j, n % 2, odd=True)

    def attn_out(j):
        st = Stats()

        def quadrant(q):
            heads = slice((q // 2) * H // 2, (q // 2 + 1) * H // 2)
            return ot[j, heads, :, quad(q)[1]].reshape(H * 16, T2)

        def emit(q, rows, v):
            r, c = quad(q, rows)
            x = xs[j, r, c] + v
            xs[j, r, c] = x
            st.add(q % 2, x)
        yield from _strassen(wo.lhs(), factors(quadrant), RC_AO, emit)
        st.save(j, twice=True)

    def mix_in(j):
        def emit(q, rows, v):
            first = quad(q, rows)[0].start
            lo = first
            while lo < first + v.shape[0]:
                hi = min(first + v.shape[0], (lo // GROUP + 1) * GROUP)
                h = _gelu_scaled(v[lo - first:hi - first])
                for a, t in enumerate(_lane_tiles(h)):
                    hs[j * NT + (q % 2) * 2 + a, lo:hi, :] = pltpu.roll(
                        t, SHIFTS[lo // GROUP] % LANE, 1)
                lo = hi
        rhs = factors(lambda q: normed(xs, j, j, 2, *quad(q)))
        yield from _strassen(w1.lhs(), rhs, RC_MI, emit)

    def mix_out(j):
        st = Stats()

        def shifted(grp, t):
            off = SHIFTS[grp]
            rows = slice(grp * GROUP, (grp + 1) * GROUP)
            lane = lax.broadcasted_iota(jnp.int32, (GROUP, LANE), 1)
            near = t - 1 if off > 0 else t + 1
            edge = lane < off if off > 0 else lane >= LANE + off
            other = hs[near, rows, :] if 0 <= near < S // LANE else jnp.zeros(lane.shape, bf16)
            return jnp.where(edge, other, hs[t, rows, :]).astype(f32)

        def quadrant(q):
            return jnp.concatenate(
                [jnp.concatenate([shifted((q // 2) * 2 + g, j * NT + (q % 2) * 2 + a) for g in range(2)],
                                 axis=0) for a in range(2)], axis=1)

        def emit(q, rows, v):
            r, c = quad(q, rows)
            x = normed(xs, j, j, 1, r, c) + v
            ys[j, r, c] = x
            st.add(q % 2, x)
        yield from _strassen(w2.lhs(), factors(quadrant, 2), RC_MO, emit)
        st.save(NB + j)

    def mlp_up(j, chunks):
        got = {}

        def emit(q, rows, v):
            got[q] = _gelu_scaled(v)
            for i, spec in enumerate(RHS_TERMS):
                if q in spec[1:] and spec[1] in got and spec[2] in got:
                    for a, t in enumerate(_lane_tiles(_term(spec, got.__getitem__))):
                        us[7 * (j % 2) + i, a, rows, :] = t
            if len(got) == 4:
                got.clear()
        rhs = factors(lambda q: normed(ys, j, NB + j, 1, *quad(q)), 1)
        yield from _strassen(w3.lhs(), rhs, chunks if w3.rows_done else RC_F_FIRST, emit)

    def mlp_down(j, chunks, last):
        st = Stats()

        def emit(q, rows, v):
            r, c = quad(q, rows)
            x = xs[j, r, c] + (ys[j, r, c] + v)
            if last:
                obuf[j, r, c] = x.astype(bf16)
                if j == NB - 1 and q in (0, 3):
                    send(j, r)
            else:
                xs[j, r, c] = x
                st.add(q % 2, x)
        yield from _strassen(w4.lhs(), lambda i: us.wide(7 * (j % 2) + i), chunks, emit)
        if last:
            if j < NB - 1:
                send(j, slice(0, D))
        else:
            st.save(j)

    def dense(plan, last):
        up, down = (RC_F_LAST, RC_DOWN_LAST) if last else (RC_F, RC_DOWN)
        stages = dict(epi=(tail, N_ATT), ao=(attn_out, 7 * len(RC_AO)),
                      mi=(mix_in, 7 * len(RC_MI)),
                      mo=(mix_out, 7 * len(RC_MO)), qk=(qkv, N_QKV),
                      up=(lambda j: mlp_up(j, up), 7 * len(up)),
                      dn=(lambda j: mlp_down(j, down, last), 7 * len(down)))

        def build(text):
            items = [(stages[w[:-1]], int(w[-1])) for w in text.split()]
            return _chain(*[f(j) for (f, _), j in items]), sum(n for (_, n), _ in items)
        for line in plan.split(";"):
            if "/" in line:
                main, side = line.split("/")
                _weave(*build(main), *build(side))
            else:
                _run(build(line)[0])

    def layer(first, last):
        _run(*[attend(0, j, None, None, j) for j in range(2)])
        if first:
            for c in w_copies[3:]:
                c.wait()

        def body(i, carry):
            for r in range(UNROLL):
                pair(i * UNROLL + r)
            return carry

        lax.fori_loop(0, (H - 1) // UNROLL, body, 0)
        dense(PLAN_LAST if last else PLAN, last)

    def x_in(j):
        st = Stats()
        for r in range(0, D, 64):
            x = xin[j, r:r + 64, :].astype(f32)
            xs[j, r:r + 64, :] = x
            st.add(0, x)
        st.save(j)

    x_copies[0].start()
    w_copies[0].start()
    clear_q()
    x_copies[0].wait()
    x_in(0)
    w_copies[0].wait()
    w_copies[1].start()
    first = qkv(0)
    for _ in range(7 * len(RC_Q)):
        next(first)
    w_copies[2].start()
    x_copies[1].start()
    w_copies[1].wait()
    for _ in range(7 * len(RC_KV)):
        next(first)
    for c in x_copies[2:]:
        c.start()
    w_copies[2].wait()
    x_copies[1].wait()
    x_in(1)
    _run(first)
    for c in w_copies[3:]:
        c.start()
    for c in x_copies[2:]:
        c.wait()
    for j in range(2, NB):
        x_in(j)
    for j in range(1, NB):
        _run(qkv(j))
    layer(True, False)
    layer(False, True)
    for c in out_copies.values():
        c.wait()


@jax.jit
def pallas_interleave_layers__mha_block__mixer_s_mlp__prompt_kernel(
    A_x: jax.Array,
    A_wqkv: jax.Array,
    A_wo: jax.Array,
    B_x: jax.Array,
    B_w1: jax.Array,
    B_w2: jax.Array,
    B_w3: jax.Array,
    B_w4: jax.Array,
):
    del B_x
    vmem = pltpu.VMEM
    out_t = pl.pallas_call(
        _kernel,
        out_shape=jax.ShapeDtypeStruct((D, S), bf16),
        in_specs=[pl.BlockSpec(memory_space=pl.ANY)] * 7,
        out_specs=pl.BlockSpec(memory_space=pl.ANY),
        scratch_shapes=[
            vmem((2, S, T), f32),
            vmem((2, 8, T), f32),
            vmem((H, S // LANE, LANE, LANE), bf16),
            vmem((4, S, LANE), bf16),
            vmem((H, S // LANE, 32, LANE), bf16),
            vmem((NB, H, 32, T), f32),
            vmem((NB, D, T), bf16),
            vmem((D, 4 * LANE), bf16),
            vmem((D, 2 * D - 4 * LANE), bf16),
            vmem((D, D), bf16),
            vmem((D, D), bf16),
            vmem((D, D), bf16),
            vmem((D, D), bf16),
            vmem((D, F), bf16),
            vmem((D, F), bf16),
            vmem((21, 2, D2, LANE), bf16),
            vmem((7, 2, D2, LANE), bf16),
            vmem((7, 2, D2, LANE), bf16),
            vmem((7, 2, D2, LANE), bf16),
            vmem((7, 2, F2, LANE), bf16),
            vmem((7, F2 // LANE, D2, LANE), bf16),
            vmem((NB, D, T), f32),
            vmem((NB, D, T), f32),
            vmem((S // LANE, D, LANE), bf16),
            vmem((14, 2, F2, LANE), bf16),
            vmem((21, 2, D2, LANE), bf16),
            vmem((D, T), f32),
            vmem((D, T), f32),
            vmem((D, T), f32),
            vmem((NB, D, T), bf16),
            vmem((2 * NB, 3, 8, T), f32),
            pltpu.SemaphoreType.DMA((NB + 8,)),
            pltpu.SemaphoreType.DMA((NB - 1 + 2 * len(RC_DOWN_LAST),)),
        ],
        compiler_params=pltpu.CompilerParams(vmem_limit_bytes=100 * 1024 * 1024),
    )(A_x.reshape(S, D).T, A_wqkv, A_wo, B_w1, B_w2, B_w3, B_w4.T)
    return out_t.T.reshape(1, S, D)
```
